```python
import os as _os
_os.environ.setdefault("JAX_PLATFORMS", "cpu")
import jax
import jax.numpy as jnp

def _softmax(x, axis=-1):
    return jax.nn.softmax(x, axis=axis)
def _gelu(x):
    return jax.nn.gelu(x, approximate=True)
def _silu(x):
    return jax.nn.silu(x)
def _sigmoid(x):
    return jax.nn.sigmoid(x)
def _layernorm(x, axis=-1, eps=1e-5):
    m = jnp.mean(x, axis=axis, keepdims=True)
    v = jnp.var(x, axis=axis, keepdims=True)
    return (x - m) / jnp.sqrt(v + eps)
def _scatter_add(tgt, idx, src, axis=0):
    return tgt.at[idx].add(src)
def _segment_sum(src, seg, n):
    return jax.ops.segment_sum(src, seg, n)
class _Rng:
    def __init__(self, key):
        self._k = key
    def _next(self):
        self._k, sub = jax.random.split(self._k)
        return sub
    def normal(self, shape):
        return jax.random.normal(self._next(), shape, dtype=jnp.bfloat16)
    def randint(self, lo, hi, shape):
        return jax.random.randint(self._next(), shape, lo, hi, dtype=jnp.int32)
    def uniform(self, shape, lo=0.0, hi=1.0):
        return jax.random.uniform(self._next(), shape, jnp.bfloat16, lo, hi)
    def permutation(self, n):
        return jax.random.permutation(self._next(), n)


kernel_name = 'sequential_preLN__softmax_full_mha__mixer_channel_mlp__prompt'

def setup_inputs():
    _rng = _Rng(jax.random.key(int.from_bytes(__import__("os").urandom(4), "little")))
    _w = (lambda a: (lambda t: t.astype(jnp.bfloat16) if jnp.issubdtype(t.dtype, jnp.floating) else t)(jnp.asarray(a)))
    def _A_setup():
        B, S, D = 1, 2048, 1024
        return {
            "x": _w((lambda *s: _rng.normal(s) * 0.05)(B, S, D)),
            "wqkv": _w((lambda *s: _rng.normal(s) * 0.05)(D, 3 * D)),
            "wo": _w((lambda *s: _rng.normal(s) * 0.05)(D, D)),
        }
    _A_in = _A_setup()

    def _B_setup():
        B, S, D, F = 1, 2048, 1024, 3584
        return {
            "x": _w((lambda *s: _rng.normal(s) * 0.05)(B, S, D)),
            "w1": _w((lambda *s: _rng.normal(s) * 0.8)(D, F) * (D ** -0.5)),
            "b1": _w((lambda *s: _rng.normal(s) * 0.8)(F)),
            "w2": _w((lambda *s: _rng.normal(s) * 0.8)(F, D) * (F ** -0.5)),
            "b2": _w((lambda *s: _rng.normal(s) * 0.05)(D)),
        }
    _B_in = _B_setup()

    return {
        "A_x": _A_in["x"],
        "A_wqkv": _A_in["wqkv"],
        "A_wo": _A_in["wo"],
        "B_x": _B_in["x"],
        "B_w1": _B_in["w1"],
        "B_b1": _B_in["b1"],
        "B_w2": _B_in["w2"],
        "B_b2": _B_in["b2"],
    }

def reference(A_x, A_wqkv, A_wo, B_x, B_w1, B_b1, B_w2, B_b2):
    def _A_ref(x, wqkv, wo):
        B, S, D = x.shape
        H = 32; Dh = D // H
        qkv = (lambda x, *d: x.transpose(*d))((x @ wqkv).reshape(B, S, 3, H, Dh), 2, 0, 3, 1, 4)
        q, k, v = qkv[0], qkv[1], qkv[2]
        scale = Dh ** -0.5
        scores = jnp.einsum("bhqd,bhkd->bhqk", q, k) * scale
        p = _softmax(scores, axis=-1)
        o = jnp.einsum("bhqk,bhkd->bhqd", p, v)
        return (lambda x, *d: x.transpose(*d))(o, 0, 2, 1, 3).reshape(B, S, D) @ wo

    def _B_ref(x, w1, b1, w2, b2):
        y = _layernorm(x, axis=-1)
        h = _gelu(jnp.einsum("bsd,df->bsf", y, w1) + b1)
        return jnp.einsum("bsf,fd->bsd", h, w2) + b2

    x = A_x
    h = x + _A_ref(_layernorm(x, axis=-1), A_wqkv, A_wo)
    h2 = h + _B_ref(_layernorm(h, axis=-1), B_w1, B_b1, B_w2, B_b2)
    return h2
```

```python
import functools
import math

import jax
import jax.numpy as jnp
from jax import lax
from jax.experimental import pallas as pl
from jax.experimental.pallas import tpu as pltpu

F32 = jnp.float32
BF16 = jnp.bfloat16

S, D, H, DH, F = 2048, 1024, 32, 32, 3584
BQ = 512
NQB = S // BQ
CK = 128
NCK = S // CK
T1 = 512
SUB1 = 256
TM = 256
FC = 512
EPS = 1e-5
QSCALE = (DH ** -0.5) * math.log2(math.e)


def _layernorm(x):
    mu = jnp.mean(x, axis=-1, keepdims=True)
    xc = x - mu
    var = jnp.mean(xc * xc, axis=-1, keepdims=True)
    return xc * lax.rsqrt(var + EPS)


def _gelu(x):
    c = math.sqrt(2.0 / math.pi)
    u = x * (c + (c * 0.044715) * (x * x))
    hx = 0.5 * x
    return hx + hx * jnp.tanh(u)


def _kernel(x_hbm, wqkv_hbm, wo_hbm, w1_hbm, b1_hbm, w2_hbm, b2_hbm, out_hbm,
            x_v, wqkv_v, wo_v, w1_v, b1_v, w2_v, b2_v,
            xn_v, k_v, qT_v, vT_v, oT_v, h_v, a_v, o_v,
            s0, s1, s2, s3, m0, m1, m2, m3, q0, q1, q2, q3,
            in_sem, out_sem):
    s_refs = (s0, s1, s2, s3)
    m_refs = (m0, m1, m2, m3)
    qm_refs = (q0, q1, q2, q3)
    n1 = S // T1

    def x_copy(t):
        return pltpu.make_async_copy(x_hbm.at[pl.ds(t * T1, T1)], x_v.at[pl.ds(t * T1, T1)], in_sem.at[t])

    def wqkv_copy(j):
        return pltpu.make_async_copy(wqkv_hbm.at[:, pl.ds(j * D, D)], wqkv_v.at[j], in_sem.at[n1 + j])

    wo_copy = pltpu.make_async_copy(wo_hbm, wo_v, in_sem.at[n1 + 3])
    w1_copy = pltpu.make_async_copy(w1_hbm, w1_v, in_sem.at[n1 + 4])
    w2_copy = pltpu.make_async_copy(w2_hbm, w2_v, in_sem.at[n1 + 5])
    b1_copy = pltpu.make_async_copy(b1_hbm, b1_v, in_sem.at[n1 + 6])
    b2_copy = pltpu.make_async_copy(b2_hbm, b2_v, in_sem.at[n1 + 7])

    x_copy(0).start()
    wqkv_copy(1).start()
    for t in range(1, n1):
        x_copy(t).start()
    wqkv_copy(0).start()
    wqkv_copy(2).start()
    wo_copy.start()
    b1_copy.start()
    b2_copy.start()
    w1_copy.start()
    w2_copy.start()

    wqkv_copy(1).wait()

    def k_body(t, carry):
        x_copy(t).wait()
        for sub in range(T1 // SUB1):
            rows = pl.ds(pl.multiple_of(t * T1 + sub * SUB1, SUB1), SUB1)
            xn = _layernorm(x_v[rows, :].astype(F32)).astype(BF16)
            xn_v[rows, :] = xn
            kk = jnp.dot(xn, wqkv_v[1], preferred_element_type=F32).astype(BF16)
            for g in range(D // 128):
                k_v[g, rows, :] = kk[:, g * 128:(g + 1) * 128]
        return carry

    lax.fori_loop(0, n1, k_body, None)

    wqkv_copy(0).wait()
    wqkv_copy(2).wait()

    def qv_body(t, carry):
        rows = pl.ds(pl.multiple_of(t * T1, T1), T1)
        xn = xn_v[rows, :]
        q = jnp.dot(xn, wqkv_v[0], preferred_element_type=F32) * QSCALE
        qT_v[t] = q.T.astype(BF16)
        v = jnp.dot(xn, wqkv_v[2], preferred_element_type=F32)
        vT_v[t] = v.T.astype(BF16)
        return carry

    lax.fori_loop(0, n1, qv_body, None)

    def put_q(h, i):
        j = h % 4
        qm_refs[i][...] = jnp.zeros((128, BQ), BF16)
        qm_refs[i][pl.ds(pl.multiple_of(j * DH, DH), DH), :] = qT_v[i, pl.ds(pl.multiple_of(h * DH, DH), DH), :]

    def qk_chunk(g, i, c, m):
        s = jnp.dot(k_v[g, pl.ds(c * CK, CK), :], qm_refs[i][...], preferred_element_type=F32)
        s_refs[i][pl.ds(c * CK, CK), :] = s
        mc = jnp.max(s.reshape(CK // 8, 8, BQ), axis=0)
        return mc if m is None else jnp.maximum(m, mc)

    def exp_chunk(i, c, m, l):
        p = jnp.exp2(s_refs[i][pl.ds(c * CK, CK), :] - m)
        for r in range(CK - 16, -1, -16):
            t = p[r:r + 8] + p[r + 8:r + 16]
            l = t if l is None else l + t
        return l, p.astype(BF16)

    def pv_chunk(h, c, p, acc):
        tb, off = divmod(c * CK, T1)
        v = vT_v[tb, pl.ds(pl.multiple_of(h * DH, DH), DH), pl.ds(off, CK)]
        o = jnp.dot(v, p, preferred_element_type=F32)
        return o if acc is None else acc + o

    def head_step(h, with_next):
        g1 = (h + 1) // 4
        for i in range(NQB):
            m_cur = jnp.max(m_refs[i][...], axis=0, keepdims=True)
            m = l = acc = None
            for c in range(NCK):
                l, p = exp_chunk(i, c, m_cur, l)
                if with_next:
                    m = qk_chunk(g1, i, c, m)
                acc = pv_chunk(h, c, p, acc)
            lsum = jnp.sum(l, axis=0, keepdims=True)
            oT_v[i, pl.ds(pl.multiple_of(h * DH, DH), DH), :] = (acc / lsum).astype(BF16)
            if with_next:
                m_refs[i][...] = m
                put_q(jnp.minimum(h + 2, H - 1), i)

    for i in range(NQB):
        put_q(0, i)
        m = None
        for c in range(NCK):
            m = qk_chunk(0, i, c, m)
        m_refs[i][...] = m
        put_q(1, i)

    def head_body(h, carry):
        head_step(h, True)
        return carry

    lax.fori_loop(0, H - 1, head_body, None)
    head_step(H - 1, False)

    wo_copy.wait()
    b1_copy.wait()
    b2_copy.wait()

    def proj_body(t, carry):
        for sub in range(T1 // SUB1):
            rows = pl.ds(pl.multiple_of(t * T1 + sub * SUB1, SUB1), SUB1)
            o = oT_v[t, :, pl.ds(sub * SUB1, SUB1)]
            attn = lax.dot_general(o, wo_v[...], (((0,), (0,)), ((), ())), preferred_element_type=F32)
            hh = x_v[rows, :].astype(F32) + attn
            xn_v[rows, :] = _layernorm(hh).astype(BF16)
            h_v[rows, :] = hh + b2_v[...].astype(F32)
        return carry

    lax.fori_loop(0, n1, proj_body, None)

    w1_copy.wait()
    w2_copy.wait()
    n3 = S // TM

    def out_copy(t):
        rows = pl.ds(pl.multiple_of(t * TM, TM), TM)
        return pltpu.make_async_copy(o_v.at[rows], out_hbm.at[rows], out_sem.at[t])

    def mlp_body(t, carry):
        rows = pl.ds(pl.multiple_of(t * TM, TM), TM)
        y = xn_v[rows, :]
        for f in range(F // FC):
            cols = pl.ds(f * FC, FC)
            z = jnp.dot(y, w1_v[:, cols], preferred_element_type=F32) + b1_v[:, cols].astype(F32)
            a_v[:, cols] = _gelu(z).astype(BF16)
        o = h_v[rows, :] + jnp.dot(a_v[...], w2_v[...], preferred_element_type=F32)
        o_v[rows, :] = o.astype(BF16)
        out_copy(t).start()
        return carry

    lax.fori_loop(0, n3, mlp_body, None)
    for t in range(n3):
        out_copy(t).wait()


@jax.jit
def pallas_sequential_preLN__softmax_full_mha__mixer_channel_mlp__prompt_kernel(
    A_x, A_wqkv, A_wo, B_x, B_w1, B_b1, B_w2, B_b2,
):
    del B_x
    any_spec = pl.BlockSpec(memory_space=pl.ANY)
    n1 = S // T1
    scratch = [
        pltpu.VMEM((S, D), BF16),
        pltpu.VMEM((3, D, D), BF16),
        pltpu.VMEM((D, D), BF16),
        pltpu.VMEM((D, F), BF16),
        pltpu.VMEM((1, F), BF16),
        pltpu.VMEM((F, D), BF16),
        pltpu.VMEM((1, D), BF16),
        pltpu.VMEM((S, D), BF16),
        pltpu.VMEM((D // 128, S, 128), BF16),
        pltpu.VMEM((NQB, D, BQ), BF16),
        pltpu.VMEM((n1, D, T1), BF16),
        pltpu.VMEM((NQB, D, BQ), BF16),
        pltpu.VMEM((S, D), F32),
        pltpu.VMEM((TM, F), BF16),
        pltpu.VMEM((S, D), BF16),
    ]
    scratch += [pltpu.VMEM((S, BQ), F32)] * NQB
    scratch += [pltpu.VMEM((8, BQ), F32)] * NQB
    scratch += [pltpu.VMEM((128, BQ), BF16)] * NQB
    scratch += [pltpu.SemaphoreType.DMA((n1 + 8,)), pltpu.SemaphoreType.DMA((S // TM,))]
    out = pl.pallas_call(
        _kernel,
        out_shape=jax.ShapeDtypeStruct((S, D), BF16),
        in_specs=[any_spec] * 7,
        out_specs=any_spec,
        scratch_shapes=scratch,
        compiler_params=pltpu.CompilerParams(vmem_limit_bytes=120 * 1024 * 1024),
        name="fused_block",
    )(A_x.reshape(S, D), A_wqkv, A_wo, B_w1, B_b1.reshape(1, F), B_w2, B_b2.reshape(1, D))
    return out.reshape(1, S, D)
```

```python
import contextlib
import functools
import math

import jax
import jax.numpy as jnp
from jax import lax
from jax.experimental import pallas as pl
from jax.experimental.pallas import tpu as pltpu

F32 = jnp.float32
BF16 = jnp.bfloat16
U32 = jnp.uint32

S, D, H, DH, F = 2048, 1024, 32, 32, 3584
D2, D4, F4 = D // 2, D // 4, F // 4
EPS = 1e-5
QSCALE = (DH ** -0.5) * math.log2(math.e)

TM = 256
NT = S // TM
RB = TM // 4
BQ = 512
NQB = S // BQ
CK = 128
NCK = S // CK
SLAB = 256
NS = D // SLAB
NU = 28
SCOPES = False


def _scope(name):
    return jax.named_scope(name) if SCOPES else contextlib.nullcontext()


def _mult(i, n):
    return i if isinstance(i, int) else pl.multiple_of(i, n)


def _pack(x):
    return pltpu.bitcast(x.astype(BF16), U32)


def _unpack(x):
    return pltpu.bitcast(x, BF16)


def _dot(a, b):
    return lax.dot_general(a, b, (((1,), (0,)), ((), ())), preferred_element_type=F32)


def _gelu(x):
    c = math.sqrt(2.0 / math.pi)
    u = x * (c + (c * 0.044715) * (x * x))
    hx = 0.5 * x
    return hx + hx * jnp.tanh(u)


class _RowNorm:
    def __init__(self, load):
        self.load = load

    def mean(self):
        self.mu = jnp.mean(self.load(), axis=-1, keepdims=True)

    def scale(self):
        xc = self.load() - self.mu
        self.rstd = lax.rsqrt(jnp.mean(xc * xc, axis=-1, keepdims=True) + EPS)

    def value(self):
        return (self.load() - self.mu) * self.rstd


def _norm_tasks(load, store):
    rows = [[pl.ds(p * 16 + r * 8, 8) for r in range(2)] for p in range(TM // 16)]
    groups = [[_RowNorm(functools.partial(load, r)) for r in pair] for pair in rows]

    def task(s):
        if s < len(groups):
            for norm in groups[s]:
                norm.mean()
        if 0 <= s - 1 < len(groups):
            for norm in groups[s - 1]:
                norm.scale()
        if s - 2 < 0:
            return []
        for r, norm in zip(rows[s - 2], groups[s - 2]):
            y = norm.value()
            store(r, y)
        return [y[:, -128:]]
    return [functools.partial(task, s) for s in range(len(groups) + 2)]


_LHS = (((0, 3), 1), ((2, 3), 1), ((0,), 0), ((3,), 0), ((0, 1), 1), ((2, 0), -1), ((1, 3), -1))
_RHS = (((0, 3), 1), ((0,), 0), ((1, 3), -1), ((2, 0), -1), ((3,), 0), ((0, 1), 1), ((2, 3), 1))


def _add(x, y):
    return [[p + q for p, q in zip(r, s)] for r, s in zip(x, y)]


def _sub(x, y):
    return [[p - q for p, q in zip(r, s)] for r, s in zip(x, y)]


def _term(table, j, quad):
    ks, sign = table[j]
    return quad(ks[0]) if sign == 0 else (_add if sign > 0 else _sub)(quad(ks[0]), quad(ks[1]))


def _terms(table, m):
    if len(m) == 1:
        return [m[0][0]]
    n = len(m) // 2
    quads = [[row[j * n:(j + 1) * n] for row in m[i * n:(i + 1) * n]] for i in (0, 1) for j in (0, 1)]
    return [t for j in range(7) for t in _terms(table, _term(table, j, quads.__getitem__))]


def _combine(product, levels, emit=None, base=0):
    if levels == 0:
        return [[product(base)]]
    step, half = 7 ** (levels - 1), 2 ** (levels - 1)

    def sub(i):
        return _combine(product, levels - 1, None, base + i * step)

    def done(r0, q0, grid):
        if emit is None:
            return grid
        return [[emit(r0 * half + r, q0 * half + q, blk) for q, blk in enumerate(row)] for r, row in enumerate(grid)]

    m3, m5 = sub(2), sub(4)
    c12 = done(0, 1, _add(m3, m5))
    m1 = sub(0)
    c22, c11 = _add(m1, m3), _sub(m1, m5)
    c22 = _add(c22, sub(5))
    c11 = _add(c11, sub(6))
    m2 = sub(1)
    c22 = done(1, 1, _sub(c22, m2))
    m4 = sub(3)
    c11 = done(0, 0, _add(c11, m4))
    c21 = done(1, 0, _add(m2, m4))
    return [r + s for r, s in zip(c11, c12)] + [r + s for r, s in zip(c21, c22)]


def _weight_term(raw, i, g):
    def quad(k):
        return raw[k // 2, :, pl.ds((k % 2) * D2 + g * 128, 128)]
    if _RHS[i][1] == 0:
        return quad(_RHS[i][0][0])
    return _term(_RHS, i, lambda k: [[quad(k).astype(F32)]])[0][0].astype(BF16)


def _weight_tasks(load, store):
    def quad(k):
        return [[load(2 * (k // 2) + r, 2 * (k % 2) + q) for q in range(2)] for r in range(2)]

    def task(j):
        for i, t in enumerate(_terms(_RHS, _term(_RHS, j, quad))):
            store(7 * j + i, _pack(t))
    return [functools.partial(task, j) for j in range(7)]


class _Filler:
    def __init__(self, tasks, slots):
        self.tasks, self.slots, self.seen, self.done, self.marks = list(tasks), slots, 0, 0, []

    def step(self):
        self.seen += 1
        want = min(len(self.tasks), -(-len(self.tasks) * self.seen // self.slots))
        marks = []
        while self.done < want:
            marks += self.tasks[self.done]() or []
            self.done += 1
        self.marks.append(marks)

    def after(self, x, lag):
        if len(self.marks) < lag or not self.marks[-lag]:
            return x
        zero = jnp.minimum(jnp.maximum(functools.reduce(jnp.maximum, self.marks[-lag]), 0.0), 0.0)
        return jnp.concatenate([x[:8] + zero, x[8:]], axis=0)

    def finish(self):
        _run(self.tasks[self.done:])
        self.done = len(self.tasks)


def _run(tasks):
    for task in tasks:
        task()


def _kernel(x_hbm, wqkv_hbm, wo_hbm, w1_hbm, b1_hbm, w2_hbm, b2_hbm, out_hbm,
            x_v, oT_v, wo_v, o_v, b1_v, b2_v, x_sem, w_sem, k_sem, u_sem, out_sem):

    def x_copy(t):
        return pltpu.make_async_copy(x_hbm.at[t], x_v.at[t], x_sem.at[t])

    def projections(k_v, qvT_v, w_v, xn_v):
        def wk_copy(s):
            cols = pl.ds(_mult(s * SLAB, SLAB), SLAB)
            return pltpu.make_async_copy(wqkv_hbm.at[:, :, pl.ds(_mult(D + s * SLAB, SLAB), SLAB)],
                                         w_v.at[1, :, :, cols], k_sem.at[s])

        def later_copies():
            return [pltpu.make_async_copy(wqkv_hbm.at[:, :, pl.ds(0, D)], w_v.at[0], w_sem.at[0]),
                    pltpu.make_async_copy(wqkv_hbm.at[:, :, pl.ds(2 * D, D)], w_v.at[2], w_sem.at[1]),
                    pltpu.make_async_copy(wo_hbm, wo_v, w_sem.at[2]),
                    pltpu.make_async_copy(b1_hbm, b1_v, w_sem.at[3]),
                    pltpu.make_async_copy(b2_hbm, b2_v, w_sem.at[4])]

        def norm_tasks(t):
            def store(rows, y):
                xn_v[t, rows, :] = y
            return _norm_tasks(lambda rows: x_v[t, rows, :].astype(F32), store)

        x_copy(0).start()
        wk_copy(0).start()

        def start_body(step, carry):
            @pl.when(step + 1 < NS)
            def _():
                wk_copy(step + 1).start()

            @pl.when(step + 1 >= NS)
            def _():
                x_copy(step + 2 - NS).start()

            @pl.when(step % (NS + 1) == 0)
            def _():
                t = step // (NS + 1)
                x_copy(t).wait()
                _run(norm_tasks(t))

            @pl.when(step % (NS + 1) != 0)
            def _():
                s = step - 1
                wk_copy(s).wait()
                kk = _dot(xn_v[0], w_v[1, :, :, pl.ds(_mult(s * SLAB, SLAB), SLAB)].reshape(D, SLAB))
                for g in range(SLAB // 128):
                    k_v[0, s * (SLAB // 128) + g] = _pack(kk[:, g * 128:(g + 1) * 128])
            return carry

        with _scope("p_start"):
            lax.fori_loop(0, NS + 2, start_body, None)

        def k_body(t, carry):
            @pl.when(t + 1 < NT)
            def _():
                x_copy(t + 1).wait()

            @pl.when(t + 3 < NT)
            def _():
                x_copy(t + 3).start()

            @pl.when(t == NT - 3)
            def _():
                for cp in later_copies():
                    cp.start()

            tasks = norm_tasks(jnp.minimum(t + 1, NT - 1))
            for rb in range(2):
                kk = _dot(xn_v[t, pl.ds(rb * (TM // 2), TM // 2), :], w_v[1].reshape(D, D))
                for g in range(D // 128):
                    k_v[t, g, pl.ds(rb * (TM // 4), TM // 4), :] = _pack(kk[:, g * 128:(g + 1) * 128])
                _run(tasks[:12] if rb == 0 else tasks[12:])
            return carry

        with _scope("p_k"):
            lax.fori_loop(1, NT, k_body, None)
        for cp in later_copies():
            cp.wait()

        def qv_body(t, carry):
            def quad(k):
                return [[xn_v[2 * t + k // 2, :, pl.ds((k % 2) * D2, D2)]]]

            for j in range(2):
                for g in range(D2 // 128):
                    def emit(r, q, blk):
                        blk = blk * QSCALE if j == 0 else blk
                        qvT_v[j, 2 * t + r, pl.ds(q * (D2 // 2) + g * 64, 64), :] = (
                            pltpu.bitcast(blk.astype(BF16).T, U32))
                    _combine(lambda i: _dot(_term(_LHS, i, quad)[0][0], _weight_term(w_v.at[2 * j], i, g)), 1, emit)
            return carry

        with _scope("p_qv"):
            lax.fori_loop(0, NT // 2, qv_body, None)

    def attention(wc, k_v, qvT_v, w1_unit, w2_unit, *bufs):
        s_refs, m_refs, q_refs = bufs[:NQB], bufs[NQB:2 * NQB], bufs[2 * NQB:]

        def unit_copies(u):
            rows = pl.ds(_mult((u % 4) * 64, 64), 64)
            copies = [pltpu.make_async_copy(
                w1_hbm.at[:, rows, pl.ds(_mult(q * F4 + (u // 4) * 128, 128), 128)],
                w1_unit.at[u % 2, q], u_sem.at[u % 2]) for q in range(4)]
            return copies + [pltpu.make_async_copy(w2_hbm.at[:, u], w2_unit.at[u % 2], u_sem.at[u % 2])]

        def w1_tasks(u, p):
            def load(r, q):
                return w1_unit[u % 2, q, r, pl.ds(p * 16, 16), :].astype(F32)

            def store(i, val):
                wc[u, i, pl.ds(p * 8, 8), :] = val
            return _weight_tasks(load, store)

        def w2_tasks(u, p, n):
            def load(r, q):
                return w2_unit[u % 2, r, pl.ds(p * 16, 16), pl.ds(q * D4 + n * 128, 128)].astype(F32)

            def store(i, val):
                wc[NU + n * (NU // 2) + u // 2, i, pl.ds(_mult((u % 2) * 16 + p * 8, 8), 8), :] = val
            return _weight_tasks(load, store)

        def weight_tasks(u):
            first = [t for p in range(4) for t in w1_tasks(u, p)]
            second = [t for p in range(2) for n in range(2) for t in w2_tasks(u, p, n)]
            return [t for pair in zip(first, second) for t in pair]

        def put_q(h, i):
            q_refs[i][...] = jnp.zeros((64, BQ), U32)
            src = pl.ds(_mult(h * (DH // 2), DH // 2), DH // 2)
            dst = pl.ds(_mult((h % 4) * (DH // 2), DH // 2), DH // 2)
            for c in range(BQ // TM):
                q_refs[i][dst, pl.ds(c * TM, TM)] = qvT_v[0, i * (BQ // TM) + c, src, :]

        def qk_chunk(keys, i, scores, c, m):
            tb, off = divmod(c * CK, TM)
            s = _dot(_unpack(keys[tb, pl.ds(off // 2, CK // 2), :]), _unpack(q_refs[i][...]))
            scores[pl.ds(c * CK, CK), :] = s
            mc = jnp.max(s.reshape(CK // 8, 8, BQ), axis=0)
            return mc if m is None else jnp.maximum(m, mc)

        def exp_chunk(i, c, m, l):
            p = jnp.exp2(s_refs[i][pl.ds(c * CK, CK), :] - m)
            for r in range(CK - 16, -1, -16):
                pair = p[r:r + 8] + p[r + 8:r + 16]
                l = pair if l is None else l + pair
            return l, p.astype(BF16)

        def pv_chunk(values, c, p, acc):
            tb, off = divmod(c * CK, TM)
            o = _dot(_unpack(values[tb, :, pl.ds(off, CK)]), p)
            return o if acc is None else acc + o

        def row_max(m):
            return jnp.broadcast_to(jnp.max(m, axis=0, keepdims=True), (8, BQ))

        def head_step(h, with_next):
            head = pl.ds(_mult(h * (DH // 2), DH // 2), DH // 2)
            values = qvT_v.at[1, :, head, :]
            result = oT_v.at[:, head, :]
            if with_next:
                keys = k_v.at[:, (h + 1) // 4]
            fill = _Filler(weight_tasks(jnp.minimum(h, NU - 1)) if with_next else [], NQB * NCK - 4)
            for i in range(NQB):
                m_cur = m_refs[i][pl.ds(0, 1), :]
                m = l = acc = None
                for c in range(NCK):
                    l, p = exp_chunk(i, c, m_cur, l)
                    if with_next:
                        m = qk_chunk(keys, i, s_refs[i], c, m)
                    acc = pv_chunk(values, c, p, acc)
                    fill.step()
                o = acc / jnp.sum(l, axis=0, keepdims=True)
                for c in range(BQ // TM):
                    result[i * (BQ // TM) + c] = _pack(o[:, c * TM:(c + 1) * TM])
                if with_next:
                    m_refs[i][...] = row_max(m)
                    put_q(jnp.minimum(h + 2, H - 1), i)
            fill.finish()

        for cp in unit_copies(0):
            cp.start()
        for i in range(NQB):
            put_q(0, i)
            m_refs[i][...] = jnp.full((8, BQ), -jnp.inf, F32)

        def first_body(cc, carry):
            keys = k_v.at[pl.ds(cc * (4 * CK // TM), 4 * CK // TM), 0]
            for i in range(NQB):
                scores = s_refs[i].at[pl.ds(_mult(cc * (4 * CK), 4 * CK), 4 * CK)]
                m = m_refs[i][...]
                for c in range(4):
                    m = qk_chunk(keys, i, scores, c, m)
                m_refs[i][...] = m
            return carry

        with _scope("p_first"):
            lax.fori_loop(0, NCK // 4, first_body, None)
        for i in range(NQB):
            put_q(1, i)
            m_refs[i][...] = row_max(m_refs[i][...])

        def head_body(h, carry):
            @pl.when(h < NU)
            def _():
                for cp in unit_copies(h):
                    cp.wait()

            @pl.when(h + 1 < NU)
            def _():
                for cp in unit_copies(h + 1):
                    cp.start()

            head_step(h, True)
            return carry

        with _scope("p_heads"):
            lax.fori_loop(0, H - 1, head_body, None)
        with _scope("p_last"):
            head_step(H - 1, False)

    def channel(wc, h_v, y_v, yt_v, act_v, lhs_v):
        def norm_tasks(t):
            def store(rows, y):
                y_v[rows, :] = y
            return _norm_tasks(lambda rows: h_v[t, rows, :], store)

        def attn_quads(t):
            o = [_unpack(oT_v[t, pl.ds(q * (D2 // 2), D2 // 2), :]).T for q in range(2)]
            return lambda k: [[o[k % 2][(k // 2) * (TM // 2):(k // 2 + 1) * (TM // 2)].astype(F32)]]

        def proj_body(t, carry):
            quad = attn_quads(jnp.minimum(t + 1, NT - 1))
            for g in range(D2 // 128):
                def product(i):
                    m = _dot(lhs_v[i], _weight_term(wo_v, i, g))
                    if g == D2 // 128 - 1:
                        lhs_v[i] = _term(_LHS, i, quad)[0][0]
                    return m

                def emit(r, q, blk):
                    rows, cols = pl.ds(r * (TM // 2), TM // 2), pl.ds(q * D2 + g * 128, 128)
                    h_v[t, rows, cols] = x_v[t, rows, cols].astype(F32) + blk
                _combine(product, 1, emit)
            return carry

        with _scope("p_proj"):
            quad = attn_quads(0)
            for i in range(7):
                lhs_v[i] = _term(_LHS, i, quad)[0][0]
            lax.fori_loop(0, NT, proj_body, None)
            _run(norm_tasks(0))

        def weight(first, count, i):
            return _unpack(wc[pl.ds(first, count), i].reshape(count * 32, 128))

        def y_term(i):
            (outer, so), (inner, si) = _LHS[i // 7], _LHS[i % 7]
            acc = None
            for a, ko in enumerate(outer):
                for b, ki in enumerate(inner):
                    r, q = 2 * (ko // 2) + ki // 2, 2 * (ko % 2) + ki % 2
                    blk = y_v[pl.ds(r * RB, RB), pl.ds(q * D4, D4)]
                    negative = (a == 1 and so < 0) != (b == 1 and si < 0)
                    acc = blk if acc is None else acc - blk if negative else acc + blk
            return acc

        def out_copy(t):
            return pltpu.make_async_copy(o_v.at[t % 2], out_hbm.at[t], out_sem.at[t % 2])

        def mlp_body(t, carry):
            @pl.when(t >= 2)
            def _():
                out_copy(t - 2).wait()

            b1 = b1_v[...].astype(F32).reshape(1, F)
            b2 = b2_v[...].astype(F32).reshape(1, D)
            for n in range(F4 // 128):
                def first(i):
                    if n == 0:
                        lhs = y_term(i)
                        yt_v[i] = _pack(lhs)
                    else:
                        lhs = _unpack(yt_v[i])
                    return _dot(lhs, weight(n * 4, 4, i))

                a = _combine(first, 2, lambda r, q, z: _gelu(z + b1[:, q * F4 + n * 128:q * F4 + (n + 1) * 128]))
                for i, term in enumerate(_terms(_LHS, a)):
                    act_v[i, :, pl.ds(n * 128, 128)] = _pack(term)
            fill = _Filler(norm_tasks(jnp.minimum(t + 1, NT - 1)), 2 * 49 - 40)
            for n in range(2):
                def second(i):
                    m = fill.after(_dot(_unpack(act_v[i]), weight(NU + n * (NU // 2), NU // 2, i)), 2)
                    fill.step()
                    return m

                def emit(r, q, z):
                    lo = q * D4 + n * 128
                    rows, cols = pl.ds(r * RB, RB), pl.ds(lo, 128)
                    o_v[t % 2, rows, cols] = (h_v[t, rows, cols] + b2[:, lo:lo + 128] + z).astype(BF16)
                _combine(second, 2, emit)
            fill.finish()
            out_copy(t).start()
            return carry

        with _scope("p_mlp"):
            lax.fori_loop(0, NT, mlp_body, None)
        with _scope("p_outwait"):
            out_copy(NT - 2).wait()
            out_copy(NT - 1).wait()

    def token_mixing(wc, k_v, qvT_v):
        pl.run_scoped(
            functools.partial(projections, k_v, qvT_v),
            pltpu.VMEM((3, 2, D2, D), BF16),
            pltpu.VMEM((NT, TM, D), F32),
        )
        pl.run_scoped(
            functools.partial(attention, wc, k_v, qvT_v),
            pltpu.VMEM((2, 4, 4, 64, 128), BF16),
            pltpu.VMEM((2, 4, 32, D), BF16),
            *([pltpu.VMEM((S, BQ), F32)] * NQB),
            *([pltpu.VMEM((8, BQ), F32)] * NQB),
            *([pltpu.VMEM((64, BQ), U32)] * NQB),
        )

    def everything(wc):
        pl.run_scoped(
            functools.partial(token_mixing, wc),
            pltpu.VMEM((NT, D // 128, TM // 2, 128), U32),
            pltpu.VMEM((2, NT, D // 2, TM), U32),
        )
        pl.run_scoped(
            functools.partial(channel, wc),
            pltpu.VMEM((NT, TM, D), F32),
            pltpu.VMEM((TM, D), F32),
            pltpu.VMEM((49, RB // 2, D4), U32),
            pltpu.VMEM((49, RB // 2, F4), U32),
            pltpu.VMEM((7, TM // 2, D2), F32),
        )

    pl.run_scoped(everything, pltpu.VMEM((2 * NU, 49, 32, 128), U32))


@jax.jit
def pallas_sequential_preLN__softmax_full_mha__mixer_channel_mlp__prompt_kernel(
    A_x: jax.Array,
    A_wqkv: jax.Array,
    A_wo: jax.Array,
    B_x: jax.Array,
    B_w1: jax.Array,
    B_b1: jax.Array,
    B_w2: jax.Array,
    B_b2: jax.Array,
):
    del B_x
    any_spec = pl.BlockSpec(memory_space=pl.ANY)
    out = pl.pallas_call(
        _kernel,
        out_shape=jax.ShapeDtypeStruct((NT, TM, D), BF16),
        in_specs=[any_spec] * 7,
        out_specs=any_spec,
        scratch_shapes=[
            pltpu.VMEM((NT, TM, D), BF16),
            pltpu.VMEM((NT, D // 2, TM), U32),
            pltpu.VMEM((2, D2, D), BF16),
            pltpu.VMEM((2, TM, D), BF16),
            pltpu.VMEM((F,), BF16),
            pltpu.VMEM((D,), BF16),
            pltpu.SemaphoreType.DMA((NT,)),
            pltpu.SemaphoreType.DMA((5,)),
            pltpu.SemaphoreType.DMA((NS,)),
            pltpu.SemaphoreType.DMA((2,)),
            pltpu.SemaphoreType.DMA((2,)),
        ],
        compiler_params=pltpu.CompilerParams(vmem_limit_bytes=112 * 1024 * 1024),
        name="fused_block",
    )(A_x.reshape(NT, TM, D), A_wqkv.reshape(2, D2, 3 * D), A_wo.reshape(2, D2, D), B_w1.reshape(4, D4, F),
      B_b1, B_w2.reshape(4, NU, 32, D), B_b2)
    return out.reshape(1, S, D)
```

```python
import functools
import math

import jax
import jax.numpy as jnp
from jax import lax
from jax.experimental import pallas as pl
from jax.experimental.pallas import tpu as pltpu

F32 = jnp.float32
BF16 = jnp.bfloat16
U32 = jnp.uint32

S, D, H, DH, F = 2048, 1024, 32, 32, 3584
D2, D4, F4 = D // 2, D // 4, F // 4
EPS = 1e-5
QSCALE = (DH ** -0.5) * math.log2(math.e)

TM = 256
NT = S // TM
RB = TM // 4
BQ = 512
NQB = S // BQ
CK = 128
NCK = S // CK
SLAB = 256
NS = D // SLAB
NU = 28


def _mult(i, n):
    return i if isinstance(i, int) else pl.multiple_of(i, n)


def _pack(x):
    return pltpu.bitcast(x.astype(BF16), U32)


def _unpack(x):
    return pltpu.bitcast(x, BF16)


def _dot(a, b):
    return lax.dot_general(a, b, (((1,), (0,)), ((), ())), preferred_element_type=F32)


def _gelu(x):
    c = math.sqrt(2.0 / math.pi)
    u = x * (c + (c * 0.044715) * (x * x))
    hx = 0.5 * x
    return hx + hx * jnp.tanh(u)


class _RowNorm:
    def __init__(self, load):
        self.load = load

    def mean(self):
        self.mu = jnp.mean(self.load(), axis=-1, keepdims=True)

    def scale(self):
        xc = self.load() - self.mu
        self.rstd = lax.rsqrt(jnp.mean(xc * xc, axis=-1, keepdims=True) + EPS)

    def value(self):
        return (self.load() - self.mu) * self.rstd


def _norm_tasks(load, store):
    rows = [[pl.ds(p * 16 + r * 8, 8) for r in range(2)] for p in range(TM // 16)]
    groups = [[_RowNorm(functools.partial(load, r)) for r in pair] for pair in rows]

    def task(s):
        if s < len(groups):
            for norm in groups[s]:
                norm.mean()
        if 0 <= s - 1 < len(groups):
            for norm in groups[s - 1]:
                norm.scale()
        if s - 2 < 0:
            return []
        for r, norm in zip(rows[s - 2], groups[s - 2]):
            y = norm.value()
            store(r, y)
        return [y[:, -128:]]
    return [functools.partial(task, s) for s in range(len(groups) + 2)]


_LHS = (((0, 3), 1), ((2, 3), 1), ((0,), 0), ((3,), 0), ((0, 1), 1), ((2, 0), -1), ((1, 3), -1))
_RHS = (((0, 3), 1), ((0,), 0), ((1, 3), -1), ((2, 0), -1), ((3,), 0), ((0, 1), 1), ((2, 3), 1))


def _add(x, y):
    return [[p + q for p, q in zip(r, s)] for r, s in zip(x, y)]


def _sub(x, y):
    return [[p - q for p, q in zip(r, s)] for r, s in zip(x, y)]


def _term(table, j, quad):
    ks, sign = table[j]
    return quad(ks[0]) if sign == 0 else (_add if sign > 0 else _sub)(quad(ks[0]), quad(ks[1]))


def _terms(table, m):
    if len(m) == 1:
        return [m[0][0]]
    n = len(m) // 2
    quads = [[row[j * n:(j + 1) * n] for row in m[i * n:(i + 1) * n]] for i in (0, 1) for j in (0, 1)]
    return [t for j in range(7) for t in _terms(table, _term(table, j, quads.__getitem__))]


def _flat_term(table, block, i):
    (outer, so), (inner, si) = table[i // 7], table[i % 7]
    acc = None
    for a, ko in enumerate(outer):
        for b, ki in enumerate(inner):
            blk = block(2 * (ko // 2) + ki // 2, 2 * (ko % 2) + ki % 2)
            negative = (a == 1 and so < 0) != (b == 1 and si < 0)
            acc = blk if acc is None else acc - blk if negative else acc + blk
    return acc


def _combine(product, levels, emit=None, base=0):
    if levels == 0:
        return [[product(base)]]
    step, half = 7 ** (levels - 1), 2 ** (levels - 1)

    def sub(i):
        return _combine(product, levels - 1, None, base + i * step)

    def done(r0, q0, grid):
        if emit is None:
            return grid
        return [[emit(r0 * half + r, q0 * half + q, blk) for q, blk in enumerate(row)] for r, row in enumerate(grid)]

    m3, m5 = sub(2), sub(4)
    c12 = done(0, 1, _add(m3, m5))
    m1 = sub(0)
    c22, c11 = _add(m1, m3), _sub(m1, m5)
    c22 = _add(c22, sub(5))
    c11 = _add(c11, sub(6))
    m2 = sub(1)
    c22 = done(1, 1, _sub(c22, m2))
    m4 = sub(3)
    c11 = done(0, 0, _add(c11, m4))
    c21 = done(1, 0, _add(m2, m4))
    return [r + s for r, s in zip(c11, c12)] + [r + s for r, s in zip(c21, c22)]


def _weight_term(raw, i, g):
    def quad(k):
        return raw[k // 2, :, pl.ds((k % 2) * D2 + g * 128, 128)]
    if _RHS[i][1] == 0:
        return quad(_RHS[i][0][0])
    return _term(_RHS, i, lambda k: [[quad(k).astype(F32)]])[0][0].astype(BF16)


def _weight_tasks(load, store):
    def quad(k):
        return [[load(2 * (k // 2) + r, 2 * (k % 2) + q) for q in range(2)] for r in range(2)]

    def task(j):
        for i, t in enumerate(_terms(_RHS, _term(_RHS, j, quad))):
            store(7 * j + i, _pack(t))
    return [functools.partial(task, j) for j in range(7)]


class _Filler:
    def __init__(self, tasks, slots):
        self.tasks, self.slots, self.seen, self.done, self.marks = list(tasks), slots, 0, 0, []

    def step(self):
        self.seen += 1
        want = min(len(self.tasks), -(-len(self.tasks) * self.seen // self.slots))
        marks = []
        while self.done < want:
            marks += self.tasks[self.done]() or []
            self.done += 1
        self.marks.append(marks)

    def after(self, x, lag):
        if len(self.marks) < lag or not self.marks[-lag]:
            return x
        zero = jnp.minimum(jnp.maximum(functools.reduce(jnp.maximum, self.marks[-lag]), 0.0), 0.0)
        return jnp.concatenate([x[:8] + zero, x[8:]], axis=0)

    def finish(self):
        _run(self.tasks[self.done:])
        self.done = len(self.tasks)


def _run(tasks):
    for task in tasks:
        task()


def _kernel(x_hbm, wqkv_hbm, wo_hbm, w1_hbm, b1_hbm, w2_hbm, b2_hbm, out_hbm,
            x_v, oT_v, wo_v, o_v, b1_v, b2_v, x_sem, w_sem, k_sem, u_sem, out_sem):

    def x_copy(t):
        return pltpu.make_async_copy(x_hbm.at[t], x_v.at[t], x_sem.at[t])

    def projections(k_v, qvT_v, w1_v, w_v, xn_v):
        def wk_copy(s):
            cols = pl.ds(_mult(s * SLAB, SLAB), SLAB)
            return pltpu.make_async_copy(wqkv_hbm.at[:, :, pl.ds(_mult(D + s * SLAB, SLAB), SLAB)],
                                         w_v.at[1, :, :, cols], k_sem.at[s])

        def later_copies():
            return [pltpu.make_async_copy(wqkv_hbm.at[:, :, pl.ds(0, D)], w_v.at[0], w_sem.at[0]),
                    pltpu.make_async_copy(wqkv_hbm.at[:, :, pl.ds(2 * D, D)], w_v.at[2], w_sem.at[1]),
                    pltpu.make_async_copy(wo_hbm, wo_v, w_sem.at[2]),
                    pltpu.make_async_copy(b1_hbm, b1_v, w_sem.at[3]),
                    pltpu.make_async_copy(b2_hbm, b2_v, w_sem.at[4])]

        def norm_tasks(t):
            def store(rows, y):
                xn_v[t, rows, :] = y
            return _norm_tasks(lambda rows: x_v[t, rows, :].astype(F32), store)

        x_copy(0).start()
        wk_copy(0).start()

        def start_body(step, carry):
            @pl.when(step + 1 < NS)
            def _():
                wk_copy(step + 1).start()

            @pl.when(step + 1 >= NS)
            def _():
                x_copy(step + 2 - NS).start()

            @pl.when(step % (NS + 1) == 0)
            def _():
                t = step // (NS + 1)
                x_copy(t).wait()
                _run(norm_tasks(t))

            @pl.when(step % (NS + 1) != 0)
            def _():
                s = step - 1
                wk_copy(s).wait()
                kk = _dot(xn_v[0], w_v[1, :, :, pl.ds(_mult(s * SLAB, SLAB), SLAB)].reshape(D, SLAB))
                for g in range(SLAB // 128):
                    k_v[0, s * (SLAB // 128) + g] = _pack(kk[:, g * 128:(g + 1) * 128])
            return carry

        lax.fori_loop(0, NS + 2, start_body, None)

        def k_body(t, carry):
            @pl.when(t + 1 < NT)
            def _():
                x_copy(t + 1).wait()

            @pl.when(t + 3 < NT)
            def _():
                x_copy(t + 3).start()

            @pl.when(t == NT - 3)
            def _():
                for cp in later_copies():
                    cp.start()

            tasks = norm_tasks(jnp.minimum(t + 1, NT - 1))
            for rb in range(2):
                kk = _dot(xn_v[t, pl.ds(rb * (TM // 2), TM // 2), :], w_v[1].reshape(D, D))
                for g in range(D // 128):
                    k_v[t, g, pl.ds(rb * (TM // 4), TM // 4), :] = _pack(kk[:, g * 128:(g + 1) * 128])
                _run(tasks[:12] if rb == 0 else tasks[12:])
            return carry

        lax.fori_loop(1, NT, k_body, None)
        for cp in later_copies():
            cp.wait()
        for n in range(F4 // 128):
            for q in range(4):
                pltpu.make_async_copy(w1_hbm.at[:, :, :, pl.ds(q * F4 + n * 128, 128)], w1_v.at[n, q],
                                      w_sem.at[5]).start()

        def qv_body(t, carry):
            def quad(k):
                return [[xn_v[2 * t + k // 2, :, pl.ds((k % 2) * D2, D2)]]]

            for j in range(2):
                for g in range(D2 // 128):
                    def emit(r, q, blk):
                        blk = blk * QSCALE if j == 0 else blk
                        qvT_v[j, 2 * t + r, pl.ds(q * (D2 // 2) + g * 64, 64), :] = (
                            pltpu.bitcast(blk.astype(BF16).T, U32))
                    _combine(lambda i: _dot(_term(_LHS, i, quad)[0][0], _weight_term(w_v.at[2 * j], i, g)), 1, emit)
            return carry

        lax.fori_loop(0, NT // 2, qv_body, None)

    def attention(wc, k_v, qvT_v, w1_v, w2_unit, *bufs):
        s_refs, m_refs, q_refs = bufs[:NQB], bufs[NQB:2 * NQB], bufs[2 * NQB:]

        def unit_copies(u):
            return [pltpu.make_async_copy(w2_hbm.at[:, u, :, pl.ds(c, D2)],
                                          w2_unit.at[u % 2, :, :, pl.ds(c, D2)], u_sem.at[u % 2]) for c in (0, D2)]

        def w1_tasks(u, p):
            def load(r, q):
                return w1_v[u // 4, q, r, u % 4, pl.ds(p * 16, 16), :].astype(F32)

            def store(i, val):
                wc[u, i, pl.ds(p * 8, 8), :] = val
            return _weight_tasks(load, store)

        def w2_tasks(u, p, n):
            def load(r, q):
                return w2_unit[u % 2, r, pl.ds(p * 16, 16), pl.ds(q * D4 + n * 128, 128)].astype(F32)

            def store(i, val):
                wc[NU + n * (NU // 2) + u // 2, i, pl.ds(_mult((u % 2) * 16 + p * 8, 8), 8), :] = val
            return _weight_tasks(load, store)

        def wo_tasks(h):
            row, n = (h // 2) * 16, h % 2

            def load(r, q):
                return wo_v[r, pl.ds(_mult(row, 16), 16), pl.ds(_mult(q * D4 + n * 128, 128), 128)].astype(F32)

            def store(i, val):
                wc[2 * NU + n * 4 + row // 64, i, pl.ds(_mult((row % 64) // 2, 8), 8), :] = val
            return _weight_tasks(load, store)

        def weight_tasks(h):
            u = jnp.minimum(h, NU - 1)
            first = [t for p in range(4) for t in w1_tasks(u, p)]
            second = [t for p in range(2) for n in range(2) for t in w2_tasks(u, p, n)]
            tasks = [t for pair in zip(second, first) for t in pair]
            for j, t in enumerate(wo_tasks(h)):
                tasks.insert(9 * j + 4, t)
            return tasks

        def put_q(h, i):
            q_refs[i][...] = jnp.zeros((64, BQ), U32)
            src = pl.ds(_mult(h * (DH // 2), DH // 2), DH // 2)
            dst = pl.ds(_mult((h % 4) * (DH // 2), DH // 2), DH // 2)
            for c in range(BQ // TM):
                q_refs[i][dst, pl.ds(c * TM, TM)] = qvT_v[0, i * (BQ // TM) + c, src, :]

        def qk_chunk(keys, i, scores, c, m):
            tb, off = divmod(c * CK, TM)
            s = _dot(_unpack(keys[tb, pl.ds(off // 2, CK // 2), :]), _unpack(q_refs[i][...]))
            scores[pl.ds(c * CK, CK), :] = s
            mc = jnp.max(s.reshape(CK // 8, 8, BQ), axis=0)
            return mc if m is None else jnp.maximum(m, mc)

        def exp_chunk(i, c, m, l):
            p = jnp.exp2(s_refs[i][pl.ds(c * CK, CK), :] - m)
            for r in range(CK - 16, -1, -16):
                pair = p[r:r + 8] + p[r + 8:r + 16]
                l = pair if l is None else l + pair
            return l, p.astype(BF16)

        def pv_chunk(values, c, p, acc):
            tb, off = divmod(c * CK, TM)
            o = _dot(_unpack(values[tb, :, pl.ds(off, CK)]), p)
            return o if acc is None else acc + o

        def row_max(m):
            return jnp.broadcast_to(jnp.max(m, axis=0, keepdims=True), (8, BQ))

        def head_step(h, with_next):
            head = pl.ds(_mult(h * (DH // 2), DH // 2), DH // 2)
            values = qvT_v.at[1, :, head, :]
            result = oT_v.at[:, head, :]
            if with_next:
                keys = k_v.at[:, (h + 1) // 4]
            fill = _Filler(weight_tasks(h) if with_next else wo_tasks(h), NQB * NCK - 1)
            for i in range(NQB):
                m_cur = m_refs[i][pl.ds(0, 1), :]
                m = l = acc = None
                for c in range(NCK):
                    l, p = exp_chunk(i, c, m_cur, l)
                    if with_next:
                        m = qk_chunk(keys, i, s_refs[i], c, m)
                    acc = pv_chunk(values, c, p, acc)
                    fill.step()
                o = acc / jnp.sum(l, axis=0, keepdims=True)
                for c in range(BQ // TM):
                    result[i * (BQ // TM) + c] = _pack(o[:, c * TM:(c + 1) * TM])
                if with_next:
                    m_refs[i][...] = row_max(m)
                    put_q(jnp.minimum(h + 2, H - 1), i)
            fill.finish()

        for cp in unit_copies(0):
            cp.start()
        for i in range(NQB):
            put_q(0, i)
            m_refs[i][...] = jnp.full((8, BQ), -jnp.inf, F32)

        def first_body(cc, carry):
            keys = k_v.at[pl.ds(cc * (4 * CK // TM), 4 * CK // TM), 0]
            for i in range(NQB):
                scores = s_refs[i].at[pl.ds(_mult(cc * (4 * CK), 4 * CK), 4 * CK)]
                m = m_refs[i][...]
                for c in range(4):
                    m = qk_chunk(keys, i, scores, c, m)
                m_refs[i][...] = m
            return carry

        lax.fori_loop(0, NCK // 4, first_body, None)
        for i in range(NQB):
            put_q(1, i)
            m_refs[i][...] = row_max(m_refs[i][...])

        pltpu.make_async_copy(w1_v, w1_v, w_sem.at[5]).wait()

        def head_body(h, carry):
            @pl.when(h < NU)
            def _():
                pltpu.make_async_copy(w2_unit.at[h % 2], w2_unit.at[h % 2], u_sem.at[h % 2]).wait()

            @pl.when(h + 1 < NU)
            def _():
                for cp in unit_copies(h + 1):
                    cp.start()

            head_step(h, True)
            return carry

        lax.fori_loop(0, H - 1, head_body, None)
        head_step(H - 1, False)

    def channel(wc, h_v, y_v, yt_v, act_v, a_v):
        def norm_tasks(t):
            def store(rows, y):
                y_v[rows, :] = y
            return _norm_tasks(lambda rows: h_v[t, rows, :], store)

        def weight(first, count, i):
            return _unpack(wc[pl.ds(first, count), i].reshape(count * 32, 128))

        def lhs_term(src, i):
            return _flat_term(_LHS, lambda r, q: src[pl.ds(r * RB, RB), pl.ds(q * D4, D4)], i)

        def stage_attention(t):
            for g in range(D // 128):
                a_v[:, pl.ds(g * 128, 128)] = _unpack(oT_v[t, pl.ds(g * 64, 64), :]).T.astype(F32)

        def proj_body(t, carry):
            for n in range(2):
                def emit(r, q, blk):
                    rows, cols = pl.ds(r * RB, RB), pl.ds(q * D4 + n * 128, 128)
                    h_v[t, rows, cols] = x_v[t, rows, cols].astype(F32) + blk
                _combine(lambda i: _dot(lhs_term(a_v, i), weight(2 * NU + n * 4, 4, i)), 2, emit)
            stage_attention(jnp.minimum(t + 1, NT - 1))
            return carry

        stage_attention(0)
        lax.fori_loop(0, NT, proj_body, None)
        _run(norm_tasks(0))

        def out_copy(t):
            return pltpu.make_async_copy(o_v.at[t % 2], out_hbm.at[t], out_sem.at[t % 2])

        def mlp_body(t, carry):
            @pl.when(t >= 2)
            def _():
                out_copy(t - 2).wait()

            b1 = b1_v[...].astype(F32).reshape(1, F)
            b2 = b2_v[...].astype(F32).reshape(1, D)
            for n in range(F4 // 128):
                def first(i):
                    if n == 0:
                        lhs = lhs_term(y_v, i)
                        yt_v[i] = _pack(lhs)
                    else:
                        lhs = _unpack(yt_v[i])
                    return _dot(lhs, weight(n * 4, 4, i))

                a = _combine(first, 2, lambda r, q, z: _gelu(z + b1[:, q * F4 + n * 128:q * F4 + (n + 1) * 128]))
                for i, term in enumerate(_terms(_LHS, a)):
                    act_v[i, :, pl.ds(n * 128, 128)] = _pack(term)
            fill = _Filler(norm_tasks(jnp.minimum(t + 1, NT - 1)), 2 * 49 - 40)
            for n in range(2):
                def second(i):
                    m = fill.after(_dot(_unpack(act_v[i]), weight(NU + n * (NU // 2), NU // 2, i)), 2)
                    fill.step()
                    return m

                def emit(r, q, z):
                    lo = q * D4 + n * 128
                    rows, cols = pl.ds(r * RB, RB), pl.ds(lo, 128)
                    o_v[t % 2, rows, cols] = (h_v[t, rows, cols] + b2[:, lo:lo + 128] + z).astype(BF16)
                _combine(second, 2, emit)
            fill.finish()
            out_copy(t).start()
            return carry

        lax.fori_loop(0, NT, mlp_body, None)
        out_copy(NT - 2).wait()
        out_copy(NT - 1).wait()

    def token_mixing(wc, k_v, qvT_v, w1_v):
        pl.run_scoped(
            functools.partial(projections, k_v, qvT_v, w1_v),
            pltpu.VMEM((3, 2, D2, D), BF16),
            pltpu.VMEM((NT, TM, D), F32),
        )
        pl.run_scoped(
            functools.partial(attention, wc, k_v, qvT_v, w1_v),
            pltpu.VMEM((2, 4, 32, D), BF16),
            *([pltpu.VMEM((S, BQ), F32)] * NQB),
            *([pltpu.VMEM((8, BQ), F32)] * NQB),
            *([pltpu.VMEM((64, BQ), U32)] * NQB),
        )

    def everything(wc):
        pl.run_scoped(
            functools.partial(token_mixing, wc),
            pltpu.VMEM((NT, D // 128, TM // 2, 128), U32),
            pltpu.VMEM((2, NT, D // 2, TM), U32),
            pltpu.VMEM((F4 // 128, 4, 4, 4, 64, 128), BF16),
        )
        pl.run_scoped(
            functools.partial(channel, wc),
            pltpu.VMEM((NT, TM, D), F32),
            pltpu.VMEM((TM, D), F32),
            pltpu.VMEM((49, RB // 2, D4), U32),
            pltpu.VMEM((49, RB // 2, F4), U32),
            pltpu.VMEM((TM, D), F32),
        )

    pl.run_scoped(everything, pltpu.VMEM((2 * NU + 8, 49, 32, 128), U32))


@jax.jit
def pallas_sequential_preLN__softmax_full_mha__mixer_channel_mlp__prompt_kernel(
    A_x: jax.Array,
    A_wqkv: jax.Array,
    A_wo: jax.Array,
    B_x: jax.Array,
    B_w1: jax.Array,
    B_b1: jax.Array,
    B_w2: jax.Array,
    B_b2: jax.Array,
):
    del B_x
    any_spec = pl.BlockSpec(memory_space=pl.ANY)
    out = pl.pallas_call(
        _kernel,
        out_shape=jax.ShapeDtypeStruct((NT, TM, D), BF16),
        in_specs=[any_spec] * 7,
        out_specs=any_spec,
        scratch_shapes=[
            pltpu.VMEM((NT, TM, D), BF16),
            pltpu.VMEM((NT, D // 2, TM), U32),
            pltpu.VMEM((4, D4, D), BF16),
            pltpu.VMEM((2, TM, D), BF16),
            pltpu.VMEM((F,), BF16),
            pltpu.VMEM((D,), BF16),
            pltpu.SemaphoreType.DMA((NT,)),
            pltpu.SemaphoreType.DMA((6,)),
            pltpu.SemaphoreType.DMA((NS,)),
            pltpu.SemaphoreType.DMA((2,)),
            pltpu.SemaphoreType.DMA((2,)),
        ],
        compiler_params=pltpu.CompilerParams(vmem_limit_bytes=112 * 1024 * 1024),
        name="fused_block",
    )(A_x.reshape(NT, TM, D), A_wqkv.reshape(2, D2, 3 * D), A_wo.reshape(4, D4, D), B_w1.reshape(4, 4, 64, F),
      B_b1, B_w2.reshape(4, NU, 32, D), B_b2)
    return out.reshape(1, S, D)
```
